```python
import jax
import jax.numpy as jnp

def _softmax(x, axis=-1):
    return jax.nn.softmax(x, axis=axis)
def _gelu(x):
    return jax.nn.gelu(x, approximate=True)
def _silu(x):
    return jax.nn.silu(x)
def _sigmoid(x):
    return jax.nn.sigmoid(x)
def _layernorm(x, axis=-1, eps=1e-5):
    m = jnp.mean(x, axis=axis, keepdims=True)
    v = jnp.var(x, axis=axis, keepdims=True)
    return (x - m) / jnp.sqrt(v + eps)
def _scatter_add(tgt, idx, src, axis=0):
    return tgt.at[idx].add(src)
def _segment_sum(src, seg, n):
    return jax.ops.segment_sum(src, seg, n)
class _Rng:
    def __init__(self, key):
        self._k = key
    def _next(self):
        self._k, sub = jax.random.split(self._k)
        return sub
    def normal(self, shape):
        return jax.random.normal(self._next(), shape, dtype=jnp.bfloat16)
    def randint(self, lo, hi, shape):
        return jax.random.randint(self._next(), shape, lo, hi, dtype=jnp.int32)
    def uniform(self, shape, lo=0.0, hi=1.0):
        return jax.random.uniform(self._next(), shape, jnp.bfloat16, lo, hi)
    def permutation(self, n):
        return jax.random.permutation(self._next(), n)


kernel_name = 'concat_heads__compressed_kv_cla__mha_block_cached__decode'

def setup_inputs():
    _rng = _Rng(jax.random.key(int.from_bytes(__import__("os").urandom(4), "little")))
    _w = (lambda a: (lambda t: t.astype(jnp.bfloat16) if jnp.issubdtype(t.dtype, jnp.floating) else t)(jnp.asarray(a)))
    def _A_setup():
        B, H, Sq, Sk, D, M = 4, 32, 1, 4096, 128, 512
        Dc = 4 * D
        return {
            "x": _w((lambda *s: _rng.normal(s) * 0.05)(B, Sq, M)),
            "c_kv": _w((lambda *s: _rng.normal(s) * 0.05)(B, Sk, Dc)),
            "w_q": _w((lambda *s: _rng.normal(s) * 0.05)(M, H, D) * (M ** -0.5)),
            "w_uk": _w((lambda *s: _rng.normal(s) * 0.05)(Dc, H, D) * (Dc ** -0.5)),
            "w_uv": _w((lambda *s: _rng.normal(s) * 0.05)(Dc, H, D) * (Dc ** -0.5)),
            "w_o": _w((lambda *s: _rng.normal(s) * 0.05)(H, D, M) * ((H * D) ** -0.5)),
        }
    _A_in = _A_setup()

    def _B_setup():
        B, Sq, D = 4, 1, 512
        H, Sk, Dh = 32, 4096, 128
        return {
            "x": _w((lambda *s: _rng.normal(s) * 0.05)(B, Sq, D)),
            "k_cache": _w((lambda *s: _rng.normal(s) * 0.05)(B, H, Sk, Dh)),
            "v_cache": _w((lambda *s: _rng.normal(s) * 0.05)(B, H, Sk, Dh)),
            "wq": _w((lambda *s: _rng.normal(s) * 0.05)(D, H * Dh) * (D ** -0.5)),
            "wo": _w((lambda *s: _rng.normal(s) * 0.05)(H * Dh, D) * ((H * Dh) ** -0.5)),
        }
    _B_in = _B_setup()

    return {
        "A_x": _A_in["x"],
        "A_c_kv": _A_in["c_kv"],
        "A_w_q": _A_in["w_q"],
        "A_w_uk": _A_in["w_uk"],
        "A_w_uv": _A_in["w_uv"],
        "A_w_o": _A_in["w_o"],
        "B_x": _B_in["x"],
        "B_k_cache": _B_in["k_cache"],
        "B_v_cache": _B_in["v_cache"],
        "B_wq": _B_in["wq"],
        "B_wo": _B_in["wo"],
    }

def reference(A_x, A_c_kv, A_w_q, A_w_uk, A_w_uv, A_w_o, B_x, B_k_cache, B_v_cache, B_wq, B_wo):
    def _A_ref(x, c_kv, w_q, w_uk, w_uv, w_o):
        B, Sq, M = x.shape[0], x.shape[1], x.shape[2]
        Sk = c_kv.shape[1]
        H, D = w_q.shape[1], w_q.shape[2]
        q = jnp.einsum("bqm,mhd->bhqd", x, w_q)
        k = jnp.einsum("bkc,chd->bhkd", c_kv, w_uk)
        v = jnp.einsum("bkc,chd->bhkd", c_kv, w_uv)
        scores = jnp.einsum("bhqd,bhkd->bhqk", q, k) * (D ** -0.5)
        off = Sk - Sq
        qi = jnp.arange(Sq)[:, None]
        kj = jnp.arange(Sk)[None, :]
        cmask = kj <= (qi + off)
        scores = jnp.where(cmask[None, None], scores, -1e9)
        p = _softmax(scores, axis=-1)
        ctx = jnp.einsum("bhqk,bhkd->bhqd", p, v)
        return jnp.einsum("bhqd,hdm->bqm", ctx, w_o)

    def _B_ref(x, k_cache, v_cache, wq, wo):
        B, Sq, D = x.shape
        H, Dh = 32, 128
        q = (lambda x, *d: x.transpose(*d))((x @ wq).reshape(B, Sq, H, Dh), 0, 2, 1, 3)
        scores = jnp.einsum("bhqd,bhkd->bhqk", q, k_cache) * (Dh ** -0.5)
        p = _softmax(scores, axis=-1)
        o = jnp.einsum("bhqk,bhkd->bhqd", p, v_cache)
        return (lambda x, *d: x.transpose(*d))(o, 0, 2, 1, 3).reshape(B, Sq, H * Dh) @ wo

    a = _A_ref(A_x, A_c_kv, A_w_q, A_w_uk, A_w_uv, A_w_o)
    b = _B_ref(B_x, B_k_cache, B_v_cache, B_wq, B_wo)
    return jnp.concatenate([a, b], axis=-1)
```

```python
import jax
import jax.numpy as jnp
import jax.experimental.pallas as pl
import jax.experimental.pallas.tpu as pltpu

_NT = (((1,), (1,)), ((), ()))

_B, _H, _D, _S, _M = 4, 32, 128, 4096, 512
_SEG = 4
_ROWS = 32
_PAIRS = 128
_CH = 512
_NC = _S // _CH
_RING = 4
_LOOK = 3
_NU = _B * _H // 8

_F32 = jnp.float32
_BF16 = jnp.bfloat16


def _kernel(xa_hbm, c_hbm, wq_hbm, wuk_hbm, wuv_hbm, woa_hbm,
            xb_hbm, k_hbm, v_hbm, wqb_hbm, wob_hbm,
            o_ref,
            xa_v, xb_v, c_v, wq_v, wuk_v, wuv_v, woa_v, wqb_v, wob_v,
            u0, u1, qabs, sa, ctxc, qb, ring, sb, pb, accb,
            wsem, rsem):

  def rows_copy(src, dst, sem, i, rows):
    r = pl.ds(pl.multiple_of(i * rows, rows), rows)
    return pltpu.make_async_copy(src.at[:, r], dst.at[:, r], sem)

  def wqb_copy(i):
    r = pl.ds(pl.multiple_of((i // 8) * 8, 8), 8)
    c = pl.ds(pl.multiple_of((i % 8) * 512, 512), 512)
    return pltpu.make_async_copy(wqb_hbm.at[:, r, c], wqb_v.at[:, r, c], wsem.at[8])

  phases = (
      (lambda i: rows_copy(wq_hbm, wq_v, wsem.at[0], i, _ROWS),
       lambda i: rows_copy(wuk_hbm, wuk_v, wsem.at[1], i, _ROWS)),
      (lambda i: rows_copy(c_hbm.at[0], c_v.at[0], wsem.at[2], i, 8),
       lambda i: rows_copy(c_hbm.at[1], c_v.at[1], wsem.at[3], i, 8)),
      (lambda i: rows_copy(c_hbm.at[2], c_v.at[2], wsem.at[4], i, 8),
       lambda i: rows_copy(c_hbm.at[3], c_v.at[3], wsem.at[5], i, 8)),
      (lambda i: rows_copy(wuv_hbm, wuv_v, wsem.at[6], i, _ROWS),
       lambda i: rows_copy(woa_hbm, woa_v, wsem.at[7], i, 8)),
      (wqb_copy,
       lambda i: rows_copy(wob_hbm, wob_v, wsem.at[9], i, 8)),
  )

  def issue(phase, start, count):
    first, second = phases[phase]

    def body(t, carry):
      for k in range(4):
        i = start + t * 4 + k
        first(i).start(priority=0)
        second(i).start(priority=1)
      return carry

    jax.lax.fori_loop(0, count // 4, body, None)

  def wait_all(buf, sem):
    pltpu.make_async_copy(buf, buf, sem).wait()

  def issue_chunk(src, unit, chunk, slot):
    def body(t, carry):
      for k in range(4):
        r = pl.multiple_of((t * 4 + k) * _ROWS, _ROWS)
        for q in range(2):
          pltpu.make_async_copy(
              src.at[unit, q, :, pl.ds(chunk * _CH + r, _ROWS)],
              ring.at[slot, q, :, pl.ds(r, _ROWS)],
              rsem.at[slot]).start(priority=q)
      return carry

    jax.lax.fori_loop(0, _CH // _ROWS // 4, body, None)

  row32 = jax.lax.broadcasted_iota(jnp.int32, (32, _D), 0) % 8
  row8 = jax.lax.broadcasted_iota(jnp.int32, (8, _D), 0)

  def replicate(x_v):
    return jnp.concatenate(
        [jnp.broadcast_to(x_v[b].astype(_F32), (8, _M)) for b in range(_B)],
        axis=0).astype(_BF16)

  def to_words(w_v, u):
    def body(t, carry):
      for s in range(_SEG):
        src = pl.ds(pl.multiple_of(t * 512, 512), 512)
        dst = pl.ds(pl.multiple_of(s * 2048 + t * 256, 256), 256)
        u[dst, :] = pltpu.bitcast(w_v[s, src, :], jnp.uint32)
      return carry

    jax.lax.fori_loop(0, 8, body, None)

  def head_pair(u, j):
    w = u[pl.ds(j, _M, stride=_H // 2), :]
    even = pltpu.bitcast(w << 16, _F32).astype(_BF16)
    odd = pltpu.bitcast(w & jnp.uint32(0xFFFF0000), _F32).astype(_BF16)
    return even, odd

  xa_copy = pltpu.make_async_copy(xa_hbm, xa_v, wsem.at[10])
  xb_copy = pltpu.make_async_copy(xb_hbm, xb_v, wsem.at[11])
  issue(0, 0, 16)
  xa_copy.start()
  xb_copy.start()
  issue(0, 16, _PAIRS - 16)

  issue(1, 0, 40)
  xa_copy.wait()
  xb_copy.wait()
  wait_all(wq_v, wsem.at[0])
  wait_all(wuk_v, wsem.at[1])
  to_words(wq_v, u0)
  issue(1, 40, 12)
  to_words(wuk_v, u1)
  issue(1, 52, 12)
  xa = replicate(xa_v)

  def absorb(g, carry):
    acc = jnp.zeros((32, _M), _F32)
    for jj in range(4):
      issue(1, 64 + g * 16 + jj * 4, 4)
      wq_pair = head_pair(u0, g * 4 + jj)
      wuk_pair = head_pair(u1, g * 4 + jj)
      for e in range(2):
        q = jnp.dot(xa, wq_pair[e], preferred_element_type=_F32)
        q = jnp.where(row32 == 2 * jj + e, q, 0.0).astype(_BF16)
        acc += jax.lax.dot_general(q, wuk_pair[e], _NT, preferred_element_type=_F32)
    for b in range(_B):
      qabs[b, pl.ds(pl.multiple_of(g * 8, 8), 8), :] = acc[b * 8:(b + 1) * 8]
    return carry

  jax.lax.fori_loop(0, 4, absorb, None)

  def latent_attention(b, issue_piece):
    qa = qabs[b].astype(_BF16)
    for s in range(_SEG):
      sa[:, s * 1024:(s + 1) * 1024] = jax.lax.dot_general(
          qa, c_v[b, s], _NT, preferred_element_type=_F32) * (_D ** -0.5)
    issue_piece(0)
    sc = sa[...]
    p = jnp.exp(sc - jnp.max(sc, axis=1, keepdims=True))
    l = jnp.sum(p, axis=1, keepdims=True)
    p = p.astype(_BF16)
    acc = jnp.zeros((_H, _M), _F32)
    for s in range(_SEG):
      acc += jnp.dot(p[:, s * 1024:(s + 1) * 1024], c_v[b, s],
                     preferred_element_type=_F32)
    acc = acc / l
    for g in range(4):
      ctxc[g, pl.ds(pl.multiple_of(b * 8, 8), 8), :] = acc[g * 8:(g + 1) * 8]
    issue_piece(1)

  def latent_pair(half, carry):
    def issue_next(start, count):
      @pl.when(half == 0)
      def _():
        issue(2, start, count)

      @pl.when(half == 1)
      def _():
        issue(3, start, count)

    issue_next(0, 48)
    for i in range(2):
      wait_all(c_v.at[half * 2 + i], wsem.at[2 + half * 2 + i])

    def one(i, c):
      latent_attention(half * 2 + i,
                       lambda piece: issue_next(48 + i * 40 + piece * 20, 20))
      return c

    jax.lax.fori_loop(0, 2, one, None)
    return carry

  jax.lax.fori_loop(0, 2, latent_pair, None)

  issue(4, 0, 48)
  wait_all(wuv_v, wsem.at[6])
  wait_all(woa_v, wsem.at[7])
  to_words(wuv_v, u0)
  issue(4, 48, 16)

  def project(g, acc):
    lat = ctxc[g].astype(_BF16)
    for jj in range(4):
      issue(4, 64 + g * 16 + jj * 4, 4)
      wuv_pair = head_pair(u0, g * 4 + jj)
      for e in range(2):
        j = 2 * jj + e
        ctx = jnp.dot(lat, wuv_pair[e], preferred_element_type=_F32)
        ctx = jnp.where(row32 == j, ctx, 0.0).astype(_BF16)
        acc += jnp.dot(ctx, woa_v[g, j * _D:(j + 1) * _D, :],
                       preferred_element_type=_F32)
    return acc

  out_a = jax.lax.fori_loop(0, 4, project, jnp.zeros((32, _M), _F32))
  for b in range(_B):
    o_ref[b, :, 0:_M] = jnp.sum(
        out_a[b * 8:(b + 1) * 8], axis=0, keepdims=True).astype(o_ref.dtype)

  for t in range(_LOOK):
    issue_chunk(k_hbm, 0, t, t)
  wait_all(wqb_v, wsem.at[8])
  wait_all(wob_v, wsem.at[9])
  xb = replicate(xb_v)
  for g in range(4):
    cols = slice(g * 1024, (g + 1) * 1024)
    q = jnp.zeros((32, 1024), _F32)
    for s in range(_SEG):
      q += jnp.dot(xb[:, s * 128:(s + 1) * 128], wqb_v[s, :, cols],
                   preferred_element_type=_F32)
    for j in range(8):
      qb[g * 8 + j] = jnp.where(row32 == j, q[:, j * _D:(j + 1) * _D], 0.0)
  accb[...] = jnp.zeros(accb.shape, _F32)

  def unit(u, carry):
    b = u // 4
    g = u % 4
    rows = pl.ds(pl.multiple_of(b * 8, 8), 8)

    def advance(t):
      n = t + _LOOK
      if n < _NC:
        issue_chunk(k_hbm, u, n, n % _RING)
      elif n < 2 * _NC:
        issue_chunk(v_hbm, u, n - _NC, n % _RING)
      else:
        @pl.when(u + 1 < _NU)
        def _():
          issue_chunk(k_hbm, u + 1, n - 2 * _NC, n % _RING)
      wait_all(ring.at[t % _RING], rsem.at[t % _RING])

    qs = [qb[g * 8 + j, rows, :].astype(_BF16) for j in range(8)]
    for t in range(_NC):
      advance(t)
      s = None
      for j in range(8):
        sj = jax.lax.dot_general(qs[j], ring[t % _RING, j // 4, j % 4], _NT,
                                 preferred_element_type=_F32)
        s = sj if s is None else s + sj
      sb[:, t * _CH:(t + 1) * _CH] = s * (_D ** -0.5)

    sc = sb[...]
    p = jnp.exp(sc - jnp.max(sc, axis=1, keepdims=True))
    l = jnp.sum(p, axis=1, keepdims=True)
    pb[...] = p

    acc = [None] * 8
    for c in range(_NC):
      t = _NC + c
      advance(t)
      pc = pb[:, c * _CH:(c + 1) * _CH].astype(_BF16)
      for j in range(8):
        o = jnp.dot(pc, ring[t % _RING, j // 4, j % 4], preferred_element_type=_F32)
        acc[j] = o if acc[j] is None else acc[j] + o

    out = accb[rows, :]
    for j in range(8):
      o = jnp.where(row8 == j, acc[j] / l, 0.0).astype(_BF16)
      out += jnp.dot(o, wob_v[g, j * _D:(j + 1) * _D, :], preferred_element_type=_F32)
    accb[rows, :] = out
    return carry

  jax.lax.fori_loop(0, _NU, unit, None)

  for b in range(_B):
    o_ref[b, :, _M:2 * _M] = jnp.sum(
        accb[b * 8:(b + 1) * 8, :], axis=0, keepdims=True).astype(o_ref.dtype)


@jax.jit
def pallas_concat_heads__compressed_kv_cla__mha_block_cached__decode_kernel(
    A_x: jax.Array,
    A_c_kv: jax.Array,
    A_w_q: jax.Array,
    A_w_uk: jax.Array,
    A_w_uv: jax.Array,
    A_w_o: jax.Array,
    B_x: jax.Array,
    B_k_cache: jax.Array,
    B_v_cache: jax.Array,
    B_wq: jax.Array,
    B_wo: jax.Array,
):
  assert A_x.shape == (_B, 1, _M) and A_c_kv.shape == (_B, _S, _M)
  assert A_w_q.shape == (_M, _H, _D) and B_k_cache.shape == (_B, _H, _S, _D)

  head_w = (_SEG, _M * _H // _SEG, _D)
  out_w = (_SEG, _H * _D // _SEG, _M)
  latent = (_B, _SEG, _S // _SEG, _M)
  cache = (_NU, 2, _SEG, _S, _D)
  wqb = (_SEG, _M // _SEG, _H * _D)

  return pl.pallas_call(
      _kernel,
      in_specs=[pl.BlockSpec(memory_space=pl.ANY)] * 11,
      out_specs=pl.BlockSpec(memory_space=pltpu.VMEM),
      out_shape=jax.ShapeDtypeStruct((_B, 1, 2 * _M), A_x.dtype),
      scratch_shapes=[
          pltpu.VMEM((_B, 1, _M), _BF16),
          pltpu.VMEM((_B, 1, _M), _BF16),
          pltpu.VMEM(latent, _BF16),
          pltpu.VMEM(head_w, _BF16),
          pltpu.VMEM(head_w, _BF16),
          pltpu.VMEM(head_w, _BF16),
          pltpu.VMEM(out_w, _BF16),
          pltpu.VMEM(wqb, _BF16),
          pltpu.VMEM(out_w, _BF16),
          pltpu.VMEM((_M * _H // 2, _D), jnp.uint32),
          pltpu.VMEM((_M * _H // 2, _D), jnp.uint32),
          pltpu.VMEM((_B, _H, _M), _F32),
          pltpu.VMEM((_H, _S), _F32),
          pltpu.VMEM((4, 32, _M), _F32),
          pltpu.VMEM((_H, 32, _D), _F32),
          pltpu.VMEM((_RING, 2, _SEG, _CH, _D), _BF16),
          pltpu.VMEM((8, _S), _F32),
          pltpu.VMEM((8, _S), _F32),
          pltpu.VMEM((32, _M), _F32),
          pltpu.SemaphoreType.DMA((12,)),
          pltpu.SemaphoreType.DMA((_RING,)),
      ],
      compiler_params=pltpu.CompilerParams(vmem_limit_bytes=100 * 1024 * 1024),
  )(
      A_x,
      A_c_kv.reshape(latent),
      A_w_q.reshape(head_w),
      A_w_uk.reshape(head_w),
      A_w_uv.reshape(head_w),
      A_w_o.reshape(out_w),
      B_x,
      B_k_cache.reshape(cache),
      B_v_cache.reshape(cache),
      B_wq.reshape(wqb),
      B_wo.reshape(out_w),
  )
```

```python
import jax
import jax.numpy as jnp
import jax.experimental.pallas as pl
import jax.experimental.pallas.tpu as pltpu

_NT = (((1,), (1,)), ((), ()))

_B, _H, _D, _S, _M = 4, 32, 128, 4096, 512
_SEG = 4
_ROWS = 32
_PAIRS = 128
_CH = 512
_NC = _S // _CH
_RING = 4
_LOOK = 3
_NU = _B * _H // 8

_F32 = jnp.float32
_BF16 = jnp.bfloat16


def _kernel(xa_hbm, c_hbm, wq_hbm, wuk_hbm, wuv_hbm, woa_hbm,
            xb_hbm, k_hbm, v_hbm, wqb_hbm, wob_hbm,
            o_ref,
            xa_v, xb_v, c_v, wq_v, wuk_v, wuv_v, woa_v, wqb_v, wob_v,
            u0, u1, qabs, sa, ctxc, qb, ring, sb, pb, accb,
            wsem, rsem):

  def rows_copy(src, dst, sem, i, rows):
    r = pl.ds(pl.multiple_of(i * rows, rows), rows)
    return pltpu.make_async_copy(src.at[:, r], dst.at[:, r], sem)

  def wqb_copy(i):
    r = pl.ds(pl.multiple_of((i // 8) * 8, 8), 8)
    c = pl.ds(pl.multiple_of((i % 8) * 512, 512), 512)
    return pltpu.make_async_copy(wqb_hbm.at[:, r, c], wqb_v.at[:, r, c], wsem.at[8])

  phases = (
      (lambda i: rows_copy(wq_hbm, wq_v, wsem.at[0], i, _ROWS),
       lambda i: rows_copy(wuk_hbm, wuk_v, wsem.at[1], i, _ROWS)),
      (lambda i: rows_copy(c_hbm.at[0], c_v.at[0], wsem.at[2], i, 8),
       lambda i: rows_copy(c_hbm.at[1], c_v.at[1], wsem.at[3], i, 8)),
      (lambda i: rows_copy(c_hbm.at[2], c_v.at[2], wsem.at[4], i, 8),
       lambda i: rows_copy(c_hbm.at[3], c_v.at[3], wsem.at[5], i, 8)),
      (lambda i: rows_copy(wuv_hbm, wuv_v, wsem.at[6], i, _ROWS),
       lambda i: rows_copy(woa_hbm, woa_v, wsem.at[7], i, 8)),
      (wqb_copy,
       lambda i: rows_copy(wob_hbm, wob_v, wsem.at[9], i, 8)),
  )

  def issue(phase, start, count):
    first, second = phases[phase]

    def body(t, carry):
      for k in range(4):
        i = start + t * 4 + k
        first(i).start(priority=0)
        second(i).start(priority=1)
      return carry

    jax.lax.fori_loop(0, count // 4, body, None)

  def wait_all(buf, sem):
    pltpu.make_async_copy(buf, buf, sem).wait()

  def issue_chunk(src, unit, chunk, slot):
    def body(t, carry):
      for k in range(4):
        r = pl.multiple_of((t * 4 + k) * _ROWS, _ROWS)
        for q in range(2):
          pltpu.make_async_copy(
              src.at[unit, q, :, pl.ds(chunk * _CH + r, _ROWS)],
              ring.at[slot, q, :, pl.ds(r, _ROWS)],
              rsem.at[slot]).start(priority=q)
      return carry

    jax.lax.fori_loop(0, _CH // _ROWS // 4, body, None)

  row32 = jax.lax.broadcasted_iota(jnp.int32, (32, _D), 0) % 8
  row8 = jax.lax.broadcasted_iota(jnp.int32, (8, _D), 0)

  def replicate(x_v):
    x = x_v[...].astype(_F32)
    return jnp.concatenate(
        [jnp.broadcast_to(x[b:b + 1], (8, _M)) for b in range(_B)],
        axis=0).astype(_BF16)

  def batch_sums(acc):
    return jnp.concatenate(
        [jnp.sum(acc[b * 8:(b + 1) * 8], axis=0, keepdims=True) for b in range(_B)],
        axis=0)

  def to_words(w_v, u):
    def body(t, carry):
      for s in range(_SEG):
        src = pl.ds(pl.multiple_of(t * 512, 512), 512)
        dst = pl.ds(pl.multiple_of(s * 1024 + t * 128, 128), 128)
        w = pltpu.bitcast(w_v[s, src, :], jnp.uint32).reshape(16, 2, 8, _D)
        for i in range(2):
          u[i, dst, :] = w[:, i].reshape(128, _D)
      return carry

    jax.lax.fori_loop(0, 8, body, None)

  def head_pair(u, g, jj):
    w = u[g // 2, pl.ds((g % 2) * 4 + jj, _M, stride=8), :]
    even = pltpu.bitcast(w << 16, _F32).astype(_BF16)
    odd = pltpu.bitcast(w & jnp.uint32(0xFFFF0000), _F32).astype(_BF16)
    return even, odd

  xa_copy = pltpu.make_async_copy(xa_hbm, xa_v, wsem.at[10])
  xb_copy = pltpu.make_async_copy(xb_hbm, xb_v, wsem.at[11])
  issue(0, 0, 16)
  xa_copy.start()
  xb_copy.start()
  issue(0, 16, _PAIRS - 16)

  issue(1, 0, 40)
  xa_copy.wait()
  xb_copy.wait()
  wait_all(wq_v, wsem.at[0])
  wait_all(wuk_v, wsem.at[1])
  to_words(wq_v, u0)
  issue(1, 40, 12)
  to_words(wuk_v, u1)
  issue(1, 52, 12)
  xa = replicate(xa_v)

  def absorb(g, carry):
    acc = jnp.zeros((32, _M), _F32)
    for jj in range(4):
      issue(1, 64 + g * 16 + jj * 4, 4)
      wq_pair = head_pair(u0, g, jj)
      wuk_pair = head_pair(u1, g, jj)
      for e in range(2):
        q = jnp.dot(xa, wq_pair[e], preferred_element_type=_F32)
        q = jnp.where(row32 == 2 * jj + e, q, 0.0).astype(_BF16)
        acc += jax.lax.dot_general(q, wuk_pair[e], _NT, preferred_element_type=_F32)
    for b in range(_B):
      qabs[b, pl.ds(pl.multiple_of(g * 8, 8), 8), :] = acc[b * 8:(b + 1) * 8]
    return carry

  jax.lax.fori_loop(0, 4, absorb, None)

  def latent_attention(b, issue_piece):
    qa = qabs[b].astype(_BF16)
    for s in range(_SEG):
      sa[:, s * 1024:(s + 1) * 1024] = jax.lax.dot_general(
          qa, c_v[b, s], _NT, preferred_element_type=_F32) * (_D ** -0.5)
    issue_piece(0)
    sc = sa[...]
    p = jnp.exp(sc - jnp.max(sc, axis=1, keepdims=True))
    l = jnp.sum(p, axis=1, keepdims=True)
    p = p.astype(_BF16)
    acc = jnp.zeros((_H, _M), _F32)
    for s in range(_SEG):
      acc += jnp.dot(p[:, s * 1024:(s + 1) * 1024], c_v[b, s],
                     preferred_element_type=_F32)
    acc = acc / l
    for g in range(4):
      ctxc[g, pl.ds(pl.multiple_of(b * 8, 8), 8), :] = acc[g * 8:(g + 1) * 8]
    issue_piece(1)

  def latent_pair(half, carry):
    def issue_next(start, count):
      @pl.when(half == 0)
      def _():
        issue(2, start, count)

      @pl.when(half == 1)
      def _():
        issue(3, start, count)

    issue_next(0, 48)
    for i in range(2):
      wait_all(c_v.at[half * 2 + i], wsem.at[2 + half * 2 + i])

    def one(i, c):
      latent_attention(half * 2 + i,
                       lambda piece: issue_next(48 + i * 40 + piece * 20, 20))
      return c

    jax.lax.fori_loop(0, 2, one, None)
    return carry

  jax.lax.fori_loop(0, 2, latent_pair, None)

  issue(4, 0, 48)
  wait_all(wuv_v, wsem.at[6])
  wait_all(woa_v, wsem.at[7])
  to_words(wuv_v, u0)
  issue(4, 48, 16)

  def project(g, acc):
    lat = ctxc[g].astype(_BF16)
    for jj in range(4):
      issue(4, 64 + g * 16 + jj * 4, 4)
      wuv_pair = head_pair(u0, g, jj)
      for e in range(2):
        j = 2 * jj + e
        ctx = jnp.dot(lat, wuv_pair[e], preferred_element_type=_F32)
        ctx = jnp.where(row32 == j, ctx, 0.0).astype(_BF16)
        acc += jnp.dot(ctx, woa_v[g, j * _D:(j + 1) * _D, :],
                       preferred_element_type=_F32)
    return acc

  out_a = jax.lax.fori_loop(0, 4, project, jnp.zeros((32, _M), _F32))
  o_ref[:, 0:_M] = batch_sums(out_a).astype(o_ref.dtype)

  for t in range(_LOOK):
    issue_chunk(k_hbm, 0, t, t)
  wait_all(wqb_v, wsem.at[8])
  wait_all(wob_v, wsem.at[9])
  xb = replicate(xb_v)
  for g in range(4):
    cols = slice(g * 1024, (g + 1) * 1024)
    q = jnp.zeros((32, 1024), _F32)
    for s in range(_SEG):
      q += jnp.dot(xb[:, s * 128:(s + 1) * 128], wqb_v[s, :, cols],
                   preferred_element_type=_F32)
    for j in range(8):
      qb[g * 8 + j] = jnp.where(row32 == j, q[:, j * _D:(j + 1) * _D], 0.0)
  accb[...] = jnp.zeros(accb.shape, _F32)

  def unit(u, carry):
    b = u // 4
    g = u % 4
    rows = pl.ds(pl.multiple_of(b * 8, 8), 8)

    def advance(t):
      n = t + _LOOK
      if n < _NC:
        issue_chunk(k_hbm, u, n, n % _RING)
      elif n < 2 * _NC:
        issue_chunk(v_hbm, u, n - _NC, n % _RING)
      else:
        @pl.when(u + 1 < _NU)
        def _():
          issue_chunk(k_hbm, u + 1, n - 2 * _NC, n % _RING)
      wait_all(ring.at[t % _RING], rsem.at[t % _RING])

    qs = [qb[g * 8 + j, rows, :].astype(_BF16) for j in range(8)]
    for t in range(_NC):
      advance(t)
      s = None
      for j in range(8):
        sj = jax.lax.dot_general(qs[j], ring[t % _RING, j // 4, j % 4], _NT,
                                 preferred_element_type=_F32)
        s = sj if s is None else s + sj
      sb[:, t * _CH:(t + 1) * _CH] = s * (_D ** -0.5)

    sc = sb[...]
    p = jnp.exp(sc - jnp.max(sc, axis=1, keepdims=True))
    l = jnp.sum(p, axis=1, keepdims=True)
    pb[...] = p

    acc = [None] * 8
    for c in range(_NC):
      t = _NC + c
      advance(t)
      pc = pb[:, c * _CH:(c + 1) * _CH].astype(_BF16)
      for j in range(8):
        o = jnp.dot(pc, ring[t % _RING, j // 4, j % 4], preferred_element_type=_F32)
        acc[j] = o if acc[j] is None else acc[j] + o

    out = accb[rows, :]
    for j in range(8):
      o = jnp.where(row8 == j, acc[j] / l, 0.0).astype(_BF16)
      out += jnp.dot(o, wob_v[g, j * _D:(j + 1) * _D, :], preferred_element_type=_F32)
    accb[rows, :] = out
    return carry

  jax.lax.fori_loop(0, _NU, unit, None)

  o_ref[:, _M:2 * _M] = batch_sums(accb[...]).astype(o_ref.dtype)


@jax.jit
def pallas_concat_heads__compressed_kv_cla__mha_block_cached__decode_kernel(
    A_x: jax.Array,
    A_c_kv: jax.Array,
    A_w_q: jax.Array,
    A_w_uk: jax.Array,
    A_w_uv: jax.Array,
    A_w_o: jax.Array,
    B_x: jax.Array,
    B_k_cache: jax.Array,
    B_v_cache: jax.Array,
    B_wq: jax.Array,
    B_wo: jax.Array,
):
  assert A_x.shape == (_B, 1, _M) and A_c_kv.shape == (_B, _S, _M)
  assert A_w_q.shape == (_M, _H, _D) and B_k_cache.shape == (_B, _H, _S, _D)

  head_w = (_SEG, _M * _H // _SEG, _D)
  out_w = (_SEG, _H * _D // _SEG, _M)
  latent = (_B, _SEG, _S // _SEG, _M)
  cache = (_NU, 2, _SEG, _S, _D)
  wqb = (_SEG, _M // _SEG, _H * _D)

  out = pl.pallas_call(
      _kernel,
      in_specs=[pl.BlockSpec(memory_space=pl.ANY)] * 11,
      out_specs=pl.BlockSpec(memory_space=pltpu.VMEM),
      out_shape=jax.ShapeDtypeStruct((_B, 2 * _M), A_x.dtype),
      scratch_shapes=[
          pltpu.VMEM((_B, _M), _BF16),
          pltpu.VMEM((_B, _M), _BF16),
          pltpu.VMEM(latent, _BF16),
          pltpu.VMEM(head_w, _BF16),
          pltpu.VMEM(head_w, _BF16),
          pltpu.VMEM(head_w, _BF16),
          pltpu.VMEM(out_w, _BF16),
          pltpu.VMEM(wqb, _BF16),
          pltpu.VMEM(out_w, _BF16),
          pltpu.VMEM((2, _M * 8, _D), jnp.uint32),
          pltpu.VMEM((2, _M * 8, _D), jnp.uint32),
          pltpu.VMEM((_B, _H, _M), _F32),
          pltpu.VMEM((_H, _S), _F32),
          pltpu.VMEM((4, 32, _M), _F32),
          pltpu.VMEM((_H, 32, _D), _F32),
          pltpu.VMEM((_RING, 2, _SEG, _CH, _D), _BF16),
          pltpu.VMEM((8, _S), _F32),
          pltpu.VMEM((8, _S), _F32),
          pltpu.VMEM((32, _M), _F32),
          pltpu.SemaphoreType.DMA((12,)),
          pltpu.SemaphoreType.DMA((_RING,)),
      ],
      compiler_params=pltpu.CompilerParams(vmem_limit_bytes=100 * 1024 * 1024),
  )(
      A_x.reshape(_B, _M),
      A_c_kv.reshape(latent),
      A_w_q.reshape(head_w),
      A_w_uk.reshape(head_w),
      A_w_uv.reshape(head_w),
      A_w_o.reshape(out_w),
      B_x.reshape(_B, _M),
      B_k_cache.reshape(cache),
      B_v_cache.reshape(cache),
      B_wq.reshape(wqb),
      B_wo.reshape(out_w),
  )
  return out.reshape(_B, 1, 2 * _M)
```

```python
import jax
import jax.numpy as jnp
import numpy as np
import jax.experimental.pallas as pl
import jax.experimental.pallas.tpu as pltpu

_NT = (((1,), (1,)), ((), ()))

_B, _H, _D, _S, _M = 4, 32, 128, 4096, 512
_SEG = 4
_ROWS = 32
_PAIRS = 128
_CH = 512
_NC = _S // _CH
_RING = 4
_LOOK = 3
_NU = _B * _H // 8

_F32 = jnp.float32
_BF16 = jnp.bfloat16


def _kernel(xa_hbm, c_hbm, wq_hbm, wuk_hbm, wuv_hbm, woa_hbm,
            xb_hbm, k_hbm, v_hbm, wqb_hbm, wob_hbm,
            o_ref,
            xa_v, xb_v, c_v, wq_v, wuk_v, wuv_v, woa_v, wqb_v, wob_v,
            u0, u1, qabs, sa, ctxc, qb, ring, sb, acc32,
            wsem, rsem):

  def rows_copy(src, dst, sem, i, rows):
    r = pl.ds(pl.multiple_of(i * rows, rows), rows)
    return pltpu.make_async_copy(src.at[:, r], dst.at[:, r], sem)

  def wqb_copy(i):
    r = pl.ds(pl.multiple_of((i // 8) * 8, 8), 8)
    c = pl.ds(pl.multiple_of((i % 8) * 512, 512), 512)
    return pltpu.make_async_copy(wqb_hbm.at[:, r, c], wqb_v.at[:, r, c], wsem.at[8])

  phases = (
      (lambda i: rows_copy(wq_hbm, wq_v, wsem.at[0], i, _ROWS),
       lambda i: rows_copy(wuk_hbm, wuk_v, wsem.at[1], i, _ROWS)),
      (lambda i: rows_copy(c_hbm.at[0], c_v.at[0], wsem.at[2], i, 8),
       lambda i: rows_copy(c_hbm.at[1], c_v.at[1], wsem.at[3], i, 8)),
      (lambda i: rows_copy(c_hbm.at[2], c_v.at[2], wsem.at[4], i, 8),
       lambda i: rows_copy(c_hbm.at[3], c_v.at[3], wsem.at[5], i, 8)),
      (lambda i: rows_copy(wuv_hbm, wuv_v, wsem.at[6], i, _ROWS),
       lambda i: rows_copy(woa_hbm, woa_v, wsem.at[7], i, 8)),
      (wqb_copy,
       lambda i: rows_copy(wob_hbm, wob_v, wsem.at[9], i, 8)),
  )

  def issue(phase, start, count):
    first, second = phases[phase]

    def body(t, carry):
      for k in range(4):
        i = start + t * 4 + k
        first(i).start(priority=0)
        second(i).start(priority=1)
      return carry

    jax.lax.fori_loop(0, count // 4, body, None)

  def wait_all(buf, sem):
    pltpu.make_async_copy(buf, buf, sem).wait()

  def issue_chunk(src, unit, chunk, slot):
    def body(t, carry):
      for k in range(4):
        r = pl.multiple_of((t * 4 + k) * _ROWS, _ROWS)
        for q in range(2):
          pltpu.make_async_copy(
              src.at[unit, q, :, pl.ds(chunk * _CH + r, _ROWS)],
              ring.at[slot, q, :, pl.ds(r, _ROWS)],
              rsem.at[slot]).start(priority=q)
      return carry

    jax.lax.fori_loop(0, _CH // _ROWS // 4, body, None)

  row32 = jax.lax.broadcasted_iota(jnp.int32, (32, _D), 0) % 8
  row8 = jax.lax.broadcasted_iota(jnp.int32, (8, _D), 0)

  def replicate(x_v):
    x = x_v[...].astype(_F32)
    return jnp.concatenate(
        [jnp.broadcast_to(x[b:b + 1], (8, _M)) for b in range(_B)],
        axis=0).astype(_BF16)

  def batch_sums(acc):
    return jnp.concatenate(
        [jnp.sum(acc[b * 8:(b + 1) * 8], axis=0, keepdims=True) for b in range(_B)],
        axis=0)

  def to_words(w_v, u):
    def body(t, carry):
      for s in range(_SEG):
        src = pl.ds(pl.multiple_of(t * 512, 512), 512)
        dst = pl.ds(pl.multiple_of(s * 1024 + t * 128, 128), 128)
        w = pltpu.bitcast(w_v[s, src, :], jnp.uint32).reshape(16, 2, 8, _D)
        for i in range(2):
          u[i, dst, :] = w[:, i].reshape(128, _D)
      return carry

    jax.lax.fori_loop(0, 8, body, None)

  def head_pair(u, j):
    w = u[j // 8, pl.ds(j % 8, _M, stride=8), :]
    even = pltpu.bitcast(w << 16, _F32).astype(_BF16)
    odd = pltpu.bitcast(w & np.uint32(0xFFFF0000), _F32).astype(_BF16)
    return even, odd

  def octet(i):
    return pl.ds(pl.multiple_of(i * 8, 8), 8)

  def head_rows(h):
    return h // 8, pl.ds(pl.multiple_of((h % 8) * _D, _D), _D)

  xa_copy = pltpu.make_async_copy(xa_hbm, xa_v, wsem.at[10])
  xb_copy = pltpu.make_async_copy(xb_hbm, xb_v, wsem.at[11])
  issue(0, 0, _PAIRS)
  xa_copy.start()
  xb_copy.start()
  acc32[...] = jnp.zeros(acc32.shape, _F32)
  for u in (u0, u1):
    u[:, _M * 8:, :] = jnp.zeros((2, 8, _D), jnp.uint32)

  issue(1, 0, 56)
  xa_copy.wait()
  xb_copy.wait()
  wait_all(wq_v, wsem.at[0])
  wait_all(wuk_v, wsem.at[1])
  to_words(wq_v, u0)
  issue(1, 56, 4)
  to_words(wuk_v, u1)
  issue(1, 60, 4)
  xa = replicate(xa_v)

  qabs[...] = jnp.zeros(qabs.shape, _F32)

  def absorb(j, carry):
    issue(1, 64 + j * 4, 4)
    wq_pair = head_pair(u0, j)
    wuk_pair = head_pair(u1, j)
    acc = qabs[j // 4]
    for e in range(2):
      q = jnp.dot(xa, wq_pair[e], preferred_element_type=_F32)
      q = jnp.where(row32 == (2 * j + e) % 8, q, 0.0).astype(_BF16)
      acc += jax.lax.dot_general(q, wuk_pair[e], _NT, preferred_element_type=_F32)
    qabs[j // 4] = acc
    return carry

  jax.lax.fori_loop(0, _H // 2, absorb, None)

  def latent_attention(b, carry):
    def issue_next(start, count):
      @pl.when(b < 2)
      def _():
        issue(2, start, count)

      @pl.when(b >= 2)
      def _():
        issue(3, start, count)

    @pl.when(b % 2 == 0)
    def _():
      issue_next(0, 64)

    wait_all(c_v.at[b], wsem.at[2 + b])
    qa = jnp.concatenate([qabs[g, octet(b), :] for g in range(4)], axis=0)
    qa = qa.astype(_BF16)

    def scores(s, m):
      issue_next(64 + (b % 2) * 32 + s * 4, 4)
      sc = jax.lax.dot_general(qa, c_v[b, s], _NT, preferred_element_type=_F32)
      sc = sc * (_D ** -0.5)
      sa[s] = sc
      return jnp.maximum(m, jnp.max(sc, axis=1, keepdims=True))

    m = jax.lax.fori_loop(0, _SEG, scores, jnp.full((_H, 1), -jnp.inf, _F32))

    def context(s, state):
      l, acc = state
      issue_next(80 + (b % 2) * 32 + s * 4, 4)
      p = jnp.exp(sa[s] - m)
      l += jnp.sum(p, axis=1, keepdims=True)
      acc += jnp.dot(p.astype(_BF16), c_v[b, s], preferred_element_type=_F32)
      return l, acc

    l, acc = jax.lax.fori_loop(
        0, _SEG, context, (jnp.zeros((_H, 1), _F32), jnp.zeros((_H, _M), _F32)))
    acc = acc / l
    for g in range(4):
      ctxc[g, octet(b), :] = acc[g * 8:(g + 1) * 8]
    return carry

  jax.lax.fori_loop(0, _B, latent_attention, None)

  issue(4, 0, 60)
  wait_all(wuv_v, wsem.at[6])
  wait_all(woa_v, wsem.at[7])
  to_words(wuv_v, u0)
  issue(4, 60, 4)

  def project(j, carry):
    issue(4, 64 + j * 4, 4)
    lat = ctxc[j // 4].astype(_BF16)
    wuv_pair = head_pair(u0, j)
    acc = acc32[...]
    for e in range(2):
      ctx = jnp.dot(lat, wuv_pair[e], preferred_element_type=_F32)
      ctx = jnp.where(row32 == (2 * j + e) % 8, ctx, 0.0).astype(_BF16)
      seg, rows = head_rows(2 * j + e)
      acc += jnp.dot(ctx, woa_v[seg, rows, :], preferred_element_type=_F32)
    acc32[...] = acc
    return carry

  jax.lax.fori_loop(0, _H // 2, project, None)
  o_ref[:, 0:_M] = batch_sums(acc32[...]).astype(o_ref.dtype)

  def prologue(t, carry):
    issue_chunk(k_hbm, 0, t, t)
    return carry

  jax.lax.fori_loop(0, _LOOK, prologue, None)
  wait_all(wqb_v, wsem.at[8])
  wait_all(wob_v, wsem.at[9])
  xb = replicate(xb_v)

  def queries(i, carry):
    cols = pl.ds(pl.multiple_of(i * 512, 512), 512)
    q = jnp.zeros((32, 512), _F32)
    for s in range(_SEG):
      q += jnp.dot(xb[:, s * 128:(s + 1) * 128], wqb_v[s, :, cols],
                   preferred_element_type=_F32)
    for j in range(4):
      qb[i * 4 + j] = jnp.where(
          row32 == (i * 4 + j) % 8, q[:, j * _D:(j + 1) * _D], 0.0)
    return carry

  jax.lax.fori_loop(0, _H // 4, queries, None)
  acc32[...] = jnp.zeros(acc32.shape, _F32)

  def unit(u, carry):
    b = u // 4
    g = u % 4

    def advance(c, src, next_src, next_unit):
      n = c + _LOOK

      @pl.when(n < _NC)
      def _():
        issue_chunk(src, u, n, n % _RING)

      @pl.when((n >= _NC) & (next_unit < _NU))
      def _():
        issue_chunk(next_src, next_unit, n - _NC, n % _RING)

      wait_all(ring.at[c % _RING], rsem.at[c % _RING])

    qs = [qb[g * 8 + j, octet(b), :].astype(_BF16) for j in range(8)]

    def scores(c, carry):
      advance(c, k_hbm, v_hbm, u)
      s = None
      for j in range(8):
        sj = jax.lax.dot_general(qs[j], ring[c % _RING, j // 4, j % 4], _NT,
                                 preferred_element_type=_F32)
        s = sj if s is None else s + sj
      sb[c] = s * (_D ** -0.5)
      return carry

    jax.lax.fori_loop(0, _NC, scores, None)

    sc = sb[...]
    m = jnp.max(jnp.max(sc, axis=0), axis=1, keepdims=True)
    p = jnp.exp(sc - m)
    l = jnp.sum(jnp.sum(p, axis=0), axis=1, keepdims=True)
    sb[...] = p / l

    def values(c, acc):
      advance(c, v_hbm, k_hbm, u + 1)
      pc = sb[c].astype(_BF16)
      for j in range(8):
        o = jnp.dot(pc, ring[c % _RING, j // 4, j % 4], preferred_element_type=_F32)
        acc += jnp.where(row8 == j, o, 0.0)
      return acc

    o = jax.lax.fori_loop(0, _NC - 1, values, jnp.zeros((8, _D), _F32))
    o = values(_NC - 1, o)

    out = acc32[octet(b), :]
    for j in range(8):
      oj = jnp.where(row8 == j, o, 0.0).astype(_BF16)
      out += jnp.dot(oj, wob_v[g, j * _D:(j + 1) * _D, :], preferred_element_type=_F32)
    acc32[octet(b), :] = out
    return carry

  jax.lax.fori_loop(0, _NU, unit, None)
  o_ref[:, _M:2 * _M] = batch_sums(acc32[...]).astype(o_ref.dtype)


@jax.jit
def pallas_concat_heads__compressed_kv_cla__mha_block_cached__decode_kernel(
    A_x: jax.Array,
    A_c_kv: jax.Array,
    A_w_q: jax.Array,
    A_w_uk: jax.Array,
    A_w_uv: jax.Array,
    A_w_o: jax.Array,
    B_x: jax.Array,
    B_k_cache: jax.Array,
    B_v_cache: jax.Array,
    B_wq: jax.Array,
    B_wo: jax.Array,
):
  assert A_x.shape == (_B, 1, _M) and A_c_kv.shape == (_B, _S, _M)
  assert A_w_q.shape == (_M, _H, _D) and B_k_cache.shape == (_B, _H, _S, _D)

  head_w = (_SEG, _M * _H // _SEG, _D)
  out_w = (_SEG, _H * _D // _SEG, _M)
  latent = (_B, _SEG, _S // _SEG, _M)
  cache = (_NU, 2, _SEG, _S, _D)
  wqb = (_SEG, _M // _SEG, _H * _D)

  out = pl.pallas_call(
      _kernel,
      in_specs=[pl.BlockSpec(memory_space=pl.ANY)] * 11,
      out_specs=pl.BlockSpec(memory_space=pltpu.VMEM),
      out_shape=jax.ShapeDtypeStruct((_B, 2 * _M), A_x.dtype),
      scratch_shapes=[
          pltpu.VMEM((_B, _M), _BF16),
          pltpu.VMEM((_B, _M), _BF16),
          pltpu.VMEM(latent, _BF16),
          pltpu.VMEM(head_w, _BF16),
          pltpu.VMEM(head_w, _BF16),
          pltpu.VMEM(head_w, _BF16),
          pltpu.VMEM(out_w, _BF16),
          pltpu.VMEM(wqb, _BF16),
          pltpu.VMEM(out_w, _BF16),
          pltpu.VMEM((2, _M * 8 + 8, _D), jnp.uint32),
          pltpu.VMEM((2, _M * 8 + 8, _D), jnp.uint32),
          pltpu.VMEM((4, 32, _M), _F32),
          pltpu.VMEM((_SEG, _H, _S // _SEG), _F32),
          pltpu.VMEM((4, 32, _M), _F32),
          pltpu.VMEM((_H, 32, _D), _F32),
          pltpu.VMEM((_RING, 2, _SEG, _CH, _D), _BF16),
          pltpu.VMEM((_NC, 8, _CH), _F32),
          pltpu.VMEM((32, _M), _F32),
          pltpu.SemaphoreType.DMA((12,)),
          pltpu.SemaphoreType.DMA((_RING,)),
      ],
      compiler_params=pltpu.CompilerParams(vmem_limit_bytes=100 * 1024 * 1024),
  )(
      A_x.reshape(_B, _M),
      A_c_kv.reshape(latent),
      A_w_q.reshape(head_w),
      A_w_uk.reshape(head_w),
      A_w_uv.reshape(head_w),
      A_w_o.reshape(out_w),
      B_x.reshape(_B, _M),
      B_k_cache.reshape(cache),
      B_v_cache.reshape(cache),
      B_wq.reshape(wqb),
      B_wo.reshape(out_w),
  )
  return out.reshape(_B, 1, 2 * _M)
```

```python
import math

import jax
import jax.numpy as jnp
import numpy as np
import jax.experimental.pallas as pl
import jax.experimental.pallas.tpu as pltpu

_NT = (((1,), (1,)), ((), ()))

_B, _H, _D, _S, _M = 4, 32, 128, 4096, 512
_SEG = 4
_ROWS = 32
_PAIRS = 128
_CH = 512
_NC = _S // _CH
_RING = _NC
_LOOK = 4
_UNROLL = 4
_NU = _B * _H // 8

_F32 = jnp.float32
_BF16 = jnp.bfloat16


def _kernel(xa_hbm, c_hbm, wq_hbm, wuk_hbm, wuv_hbm, woa_hbm,
            xb_hbm, k_hbm, v_hbm, wqb_hbm, wob_hbm,
            o_ref,
            x_v, wqk_v, c_v, wuv_v, wqb_v, ring, wo_v,
            u0, u1, qabs, sa, ctxc, qb, sb, heads,
            sems):

  wqk_sem, x_sem = sems.at[0], sems.at[1]
  wuv_sem, wqb_sem = sems.at[_RING - 2], sems.at[_RING - 1]

  def latent_sem(half):
    return sems.at[_RING - 4 + half]

  def rows_copy(src, dst, sem, i, rows):
    r = pl.ds(pl.multiple_of(i * rows, rows), rows)
    return pltpu.make_async_copy(src.at[:, r], dst.at[:, r], sem)

  def wqb_copy(i):
    r = pl.ds(pl.multiple_of((i // 8) * 8, 8), 8)
    c = pl.ds(pl.multiple_of((i % 8) * 512, 512), 512)
    return pltpu.make_async_copy(wqb_hbm.at[:, r, c], wqb_v.at[:, r, c], wqb_sem)

  phases = (
      (lambda i: rows_copy(wq_hbm, wqk_v.at[0], wqk_sem, i, _ROWS),
       lambda i: rows_copy(wuk_hbm, wqk_v.at[1], wqk_sem, i, _ROWS)),
      (lambda i: rows_copy(c_hbm.at[0], c_v.at[0], latent_sem(0), i, 8),
       lambda i: rows_copy(c_hbm.at[1], c_v.at[1], latent_sem(0), i, 8)),
      (lambda i: rows_copy(c_hbm.at[2], c_v.at[2], latent_sem(1), i, 8),
       lambda i: rows_copy(c_hbm.at[3], c_v.at[3], latent_sem(1), i, 8)),
      (lambda i: rows_copy(wuv_hbm, wuv_v, wuv_sem, i, _ROWS),
       wqb_copy),
  )

  def issue_pairs(pair, start, count):
    step = math.gcd(count, _UNROLL)

    def body(t, carry):
      for k in range(step):
        for queue, copy in enumerate(pair(start + t * step + k)):
          copy.start(priority=queue)
      return carry

    if step == count:
      body(0, None)
    else:
      jax.lax.fori_loop(0, count // step, body, None)

  def issue(phase, start, count):
    issue_pairs(lambda i: [copy(i) for copy in phases[phase]], start, count)

  def issue_chunk(src, unit, chunk):
    def pair(i):
      r = pl.multiple_of(i * _ROWS, _ROWS)
      return [
          pltpu.make_async_copy(
              src.at[unit, q, :, pl.ds(chunk * _CH + r, _ROWS)],
              ring.at[chunk, q, :, pl.ds(r, _ROWS)], sems.at[chunk])
          for q in range(2)
      ]

    issue_pairs(pair, 0, _CH // _ROWS)

  def issue_out_chunk(j):
    def pair(i):
      return [rows_copy(src, wo_v.at[q], sems.at[j], i, 8)
              for q, src in enumerate((woa_hbm, wob_hbm))]

    issue_pairs(pair, j * 16, 16)

  def wait_all(buf, sem):
    pltpu.make_async_copy(buf, buf, sem).wait()

  row32 = jax.lax.broadcasted_iota(jnp.int32, (32, _D), 0) % 8
  row8 = jax.lax.broadcasted_iota(jnp.int32, (8, _D), 0)

  def replicate(x):
    x = x.astype(_F32)
    return jnp.concatenate(
        [jnp.broadcast_to(x[b:b + 1], (8, _M)) for b in range(_B)],
        axis=0).astype(_BF16)

  def batch_sums(acc):
    return jnp.concatenate(
        [jnp.sum(acc[b * 8:(b + 1) * 8], axis=0, keepdims=True) for b in range(_B)],
        axis=0)

  def to_words(w_v, u):
    def body(t, carry):
      for s in range(_SEG):
        src = pl.ds(pl.multiple_of(t * 512, 512), 512)
        dst = pl.ds(pl.multiple_of(s * 1024 + t * 128, 128), 128)
        w = pltpu.bitcast(w_v[s, src, :], jnp.uint32).reshape(16, 2, 8, _D)
        for i in range(2):
          u[i, dst, :] = w[:, i].reshape(128, _D)
      return carry

    jax.lax.fori_loop(0, 8, body, None)

  def head_pair(u, j):
    w = u[j // 8, pl.ds(j % 8, _M, stride=8), :]
    even = pltpu.bitcast(w << 16, _F32).astype(_BF16)
    odd = pltpu.bitcast(w & np.uint32(0xFFFF0000), _F32).astype(_BF16)
    return even, odd

  def octet(i):
    return pl.ds(pl.multiple_of(i * 8, 8), 8)

  x_copies = [pltpu.make_async_copy(x_hbm, x_v.at[i], x_sem)
              for i, x_hbm in enumerate((xa_hbm, xb_hbm))]
  issue(0, 0, _PAIRS)
  for copy in x_copies:
    copy.start()
  for u in (u0, u1):
    u[:, _M * 8:, :] = jnp.zeros((2, 8, _D), jnp.uint32)

  issue(1, 0, 56)
  for copy in x_copies:
    copy.wait()
  wait_all(wqk_v, wqk_sem)
  to_words(wqk_v.at[0], u0)
  issue(1, 56, 4)
  to_words(wqk_v.at[1], u1)
  issue(1, 60, 4)
  xa = replicate(x_v[0])

  qabs[...] = jnp.zeros(qabs.shape, _F32)

  def absorb(j, carry):
    issue(1, 64 + j * 4, 4)
    wq_pair = head_pair(u0, j)
    wuk_pair = head_pair(u1, j)
    acc = qabs[j // 4]
    for e in range(2):
      q = jnp.dot(xa, wq_pair[e], preferred_element_type=_F32)
      q = jnp.where(row32 == (2 * j + e) % 8, q, 0.0).astype(_BF16)
      acc += jax.lax.dot_general(q, wuk_pair[e], _NT, preferred_element_type=_F32)
    qabs[j // 4] = acc
    return carry

  jax.lax.fori_loop(0, _H // 2, absorb, None)

  def latent_attention(b, carry):
    def issue_next(start, count):
      @pl.when(b < 2)
      def _():
        issue(2, start, count)

      @pl.when(b >= 2)
      def _():
        issue(3, start, count)

    @pl.when(b % 2 == 0)
    def _():
      issue_next(0, 64)
      wait_all(c_v.at[pl.ds(b, 2)], latent_sem(b // 2))

    qa = jnp.concatenate([qabs[g, octet(b), :] for g in range(4)], axis=0)
    qa = qa.astype(_BF16)

    def scores(s, m):
      issue_next(64 + (b % 2) * 32 + s * 4, 4)
      sc = jax.lax.dot_general(qa, c_v[b, s], _NT, preferred_element_type=_F32)
      sc = sc * (_D ** -0.5)
      sa[s] = sc
      return jnp.maximum(m, jnp.max(sc, axis=1, keepdims=True))

    m = jax.lax.fori_loop(0, _SEG, scores, jnp.full((_H, 1), -jnp.inf, _F32))

    def context(s, state):
      l, acc = state
      issue_next(80 + (b % 2) * 32 + s * 4, 4)
      p = jnp.exp(sa[s] - m)
      l += jnp.sum(p, axis=1, keepdims=True)
      acc += jnp.dot(p.astype(_BF16), c_v[b, s], preferred_element_type=_F32)
      return l, acc

    l, acc = jax.lax.fori_loop(
        0, _SEG, context, (jnp.zeros((_H, 1), _F32), jnp.zeros((_H, _M), _F32)))
    acc = acc / l
    for g in range(4):
      ctxc[g, octet(b), :] = acc[g * 8:(g + 1) * 8]
    return carry

  jax.lax.fori_loop(0, _B, latent_attention, None)

  heads[0] = jnp.zeros(heads.shape[1:], _F32)

  def up_project(j):
    lat = ctxc[j // 4].astype(_BF16)
    wuv_pair = head_pair(u0, j)
    ctx = heads[0, j // 4]
    for e in range(2):
      new = jnp.dot(lat, wuv_pair[e], preferred_element_type=_F32)
      ctx = jnp.where(row32 == (2 * j + e) % 8, new, ctx)
    heads[0, j // 4] = ctx

  def prologue(t, carry):
    issue_chunk(k_hbm, 0, t)
    return carry

  jax.lax.fori_loop(0, _LOOK, prologue, None)
  wait_all(wuv_v, wuv_sem)
  wait_all(wqb_v, wqb_sem)
  to_words(wuv_v, u0)
  xb = replicate(x_v[1])

  def queries(i, carry):
    cols = pl.ds(pl.multiple_of(i * 512, 512), 512)
    q = jnp.zeros((32, 512), _F32)
    for s in range(_SEG):
      q += jnp.dot(xb[:, s * 128:(s + 1) * 128], wqb_v[s, :, cols],
                   preferred_element_type=_F32)
    for j in range(4):
      qb[i * 4 + j] = jnp.where(
          row32 == (i * 4 + j) % 8, q[:, j * _D:(j + 1) * _D], 0.0)
    return carry

  jax.lax.fori_loop(0, _H // 4, queries, None)

  def unit(u, carry):
    b = u // 4
    g = u % 4

    def advance(c, src, issue_following):
      n = c + _LOOK

      @pl.when(n < _NC)
      def _():
        issue_chunk(src, u, n)

      @pl.when(n >= _NC)
      def _():
        issue_following(n - _NC)

      wait_all(ring.at[c], sems.at[c])

    def after_scores(c):
      issue_chunk(v_hbm, u, c)

    def after_values(c):
      @pl.when(u + 1 < _NU)
      def _():
        issue_chunk(k_hbm, u + 1, c)

      @pl.when(u + 1 == _NU)
      def _():
        issue_out_chunk(c)

    qs = [qb[g * 8 + j, octet(b), :].astype(_BF16) for j in range(8)]

    def scores(c, carry):
      advance(c, k_hbm, after_scores)
      s = None
      for j in range(8):
        sj = jax.lax.dot_general(qs[j], ring[c, j // 4, j % 4], _NT,
                                 preferred_element_type=_F32)
        s = sj if s is None else s + sj
      sb[c] = s * (_D ** -0.5)
      return carry

    jax.lax.fori_loop(0, _NC, scores, None)

    sc = sb[...]
    m = jnp.max(jnp.max(sc, axis=0), axis=1, keepdims=True)
    p = jnp.exp(sc - m)
    l = jnp.sum(jnp.sum(p, axis=0), axis=1, keepdims=True)
    sb[...] = p / l

    def values(c, acc):
      advance(c, v_hbm, after_values)
      pc = sb[c].astype(_BF16)
      for j in range(8):
        o = jnp.dot(pc, ring[c, j // 4, j % 4], preferred_element_type=_F32)
        acc += jnp.where(row8 == j, o, 0.0)
      return acc

    up_project(u)
    heads[1, g, octet(b), :] = jax.lax.fori_loop(
        0, _NC, values, jnp.zeros((8, _D), _F32))
    return carry

  jax.lax.fori_loop(0, _NU, unit, None)

  def out_project(j, accs):
    @pl.when(j + _LOOK < 8)
    def _():
      issue_out_chunk(j + _LOOK)

    rows = pl.ds(pl.multiple_of(j * _D, _D), _D)
    wait_all(wo_v.at[:, :, rows], sems.at[j])
    out = []
    for q, acc in enumerate(accs):
      for g in range(4):
        lhs = jnp.where(row32 == j, heads[q, g], 0.0).astype(_BF16)
        acc += jnp.dot(lhs, wo_v[q, g, rows, :], preferred_element_type=_F32)
      out.append(acc)
    return tuple(out)

  zero = jnp.zeros((32, _M), _F32)
  for q, acc in enumerate(jax.lax.fori_loop(0, 8, out_project, (zero, zero))):
    o_ref[:, q * _M:(q + 1) * _M] = batch_sums(acc).astype(o_ref.dtype)


@jax.jit
def pallas_concat_heads__compressed_kv_cla__mha_block_cached__decode_kernel(
    A_x: jax.Array,
    A_c_kv: jax.Array,
    A_w_q: jax.Array,
    A_w_uk: jax.Array,
    A_w_uv: jax.Array,
    A_w_o: jax.Array,
    B_x: jax.Array,
    B_k_cache: jax.Array,
    B_v_cache: jax.Array,
    B_wq: jax.Array,
    B_wo: jax.Array,
):
  assert A_x.shape == (_B, 1, _M) and A_c_kv.shape == (_B, _S, _M)
  assert A_w_q.shape == (_M, _H, _D) and B_k_cache.shape == (_B, _H, _S, _D)

  head_w = (_SEG, _M * _H // _SEG, _D)
  out_w = (_SEG, _H * _D // _SEG, _M)
  latent = (_B, _SEG, _S // _SEG, _M)
  cache = (_NU, 2, _SEG, _S, _D)
  wqb = (_SEG, _M // _SEG, _H * _D)

  out = pl.pallas_call(
      _kernel,
      in_specs=[pl.BlockSpec(memory_space=pl.ANY)] * 11,
      out_specs=pl.BlockSpec(memory_space=pltpu.VMEM),
      out_shape=jax.ShapeDtypeStruct((_B, 2 * _M), A_x.dtype),
      scratch_shapes=[
          pltpu.VMEM((2, _B, _M), _BF16),
          pltpu.VMEM((2,) + head_w, _BF16),
          pltpu.VMEM(latent, _BF16),
          pltpu.VMEM(head_w, _BF16),
          pltpu.VMEM(wqb, _BF16),
          pltpu.VMEM((_RING, 2, _SEG, _CH, _D), _BF16),
          pltpu.VMEM((2,) + out_w, _BF16),
          pltpu.VMEM((2, _M * 8 + 8, _D), jnp.uint32),
          pltpu.VMEM((2, _M * 8 + 8, _D), jnp.uint32),
          pltpu.VMEM((4, 32, _M), _F32),
          pltpu.VMEM((_SEG, _H, _S // _SEG), _F32),
          pltpu.VMEM((4, 32, _M), _F32),
          pltpu.VMEM((_H, 32, _D), _F32),
          pltpu.VMEM((_NC, 8, _CH), _F32),
          pltpu.VMEM((2, 4, 32, _D), _F32),
          pltpu.SemaphoreType.DMA((_RING,)),
      ],
      compiler_params=pltpu.CompilerParams(vmem_limit_bytes=100 * 1024 * 1024),
  )(
      A_x.reshape(_B, _M),
      A_c_kv.reshape(latent),
      A_w_q.reshape(head_w),
      A_w_uk.reshape(head_w),
      A_w_uv.reshape(head_w),
      A_w_o.reshape(out_w),
      B_x.reshape(_B, _M),
      B_k_cache.reshape(cache),
      B_v_cache.reshape(cache),
      B_wq.reshape(wqb),
      B_wo.reshape(out_w),
  )
  return out.reshape(_B, 1, 2 * _M)
```
